```python
import os as _os
_os.environ.setdefault("JAX_PLATFORMS", "cpu")
import jax
import jax.numpy as jnp

def _softmax(x, axis=-1):
    return jax.nn.softmax(x, axis=axis)
def _gelu(x):
    return jax.nn.gelu(x, approximate=True)
def _silu(x):
    return jax.nn.silu(x)
def _sigmoid(x):
    return jax.nn.sigmoid(x)
def _layernorm(x, axis=-1, eps=1e-5):
    m = jnp.mean(x, axis=axis, keepdims=True)
    v = jnp.var(x, axis=axis, keepdims=True)
    return (x - m) / jnp.sqrt(v + eps)
def _scatter_add(tgt, idx, src, axis=0):
    return tgt.at[idx].add(src)
def _segment_sum(src, seg, n):
    return jax.ops.segment_sum(src, seg, n)
class _Rng:
    def __init__(self, key):
        self._k = key
    def _next(self):
        self._k, sub = jax.random.split(self._k)
        return sub
    def normal(self, shape):
        return jax.random.normal(self._next(), shape, dtype=jnp.bfloat16)
    def randint(self, lo, hi, shape):
        return jax.random.randint(self._next(), shape, lo, hi, dtype=jnp.int32)
    def uniform(self, shape, lo=0.0, hi=1.0):
        return jax.random.uniform(self._next(), shape, jnp.bfloat16, lo, hi)
    def permutation(self, n):
        return jax.random.permutation(self._next(), n)


kernel_name = 'sequential_preLN__sliding_block__dense_activation_relu__prompt'

def setup_inputs():
    _rng = _Rng(jax.random.key(int.from_bytes(__import__("os").urandom(4), "little")))
    _w = (lambda a: (lambda t: t.astype(jnp.bfloat16) if jnp.issubdtype(t.dtype, jnp.floating) else t)(jnp.asarray(a)))
    def _A_setup():
        B, S, D = 1, 2048, 640
        return {
            "x": _w((lambda *s: _rng.normal(s) * 0.05)(B, S, D)),
            "wqkv": _w((lambda *s: _rng.normal(s) * 0.05)(D, 3 * D)),
            "wo": _w((lambda *s: _rng.normal(s) * 0.05)(D, D)),
        }
    _A_in = _A_setup()

    def _B_setup():
        B, S, D, Dff = 1, 2048, 640, 1536
        return {
            "x": _w((lambda *s: _rng.normal(s) * 0.05)(B, S, D)),
            "w1": _w((lambda *s: _rng.normal(s) * 0.05)(D, Dff)),
            "w2": _w((lambda *s: _rng.normal(s) * 0.05)(Dff, D)),
        }
    _B_in = _B_setup()

    return {
        "A_x": _A_in["x"],
        "A_wqkv": _A_in["wqkv"],
        "A_wo": _A_in["wo"],
        "B_x": _B_in["x"],
        "B_w1": _B_in["w1"],
        "B_w2": _B_in["w2"],
    }

def reference(A_x, A_wqkv, A_wo, B_x, B_w1, B_w2):
    def _A_ref(x, wqkv, wo):
        B, S, D = x.shape
        H = 32; Dh = D // H; W = 256
        qkv = (lambda x, *d: x.transpose(*d))((x @ wqkv).reshape(B, S, 3, H, Dh), 2, 0, 3, 1, 4)
        q, k, v = qkv[0], qkv[1], qkv[2]
        scores = jnp.einsum("bhqd,bhkd->bhqk", q, k) * (Dh ** -0.5)
        idx = jnp.arange(S)
        mask = (idx[:, None] - idx[None, :] >= 0) & (idx[:, None] - idx[None, :] < W)
        scores = jnp.where(mask[None, None], scores, -1e9)
        p = _softmax(scores, axis=-1)
        o = jnp.einsum("bhqk,bhkd->bhqd", p, v)
        return (lambda x, *d: x.transpose(*d))(o, 0, 2, 1, 3).reshape(B, S, D) @ wo

    def _B_ref(x, w1, w2):
        h = jnp.einsum("bsd,df->bsf", x, w1)
        zero = jnp.zeros_like(h)
        h = jnp.maximum(h, zero)
        return jnp.einsum("bsf,fd->bsd", h, w2)

    x = A_x
    h = x + _A_ref(_layernorm(x, axis=-1), A_wqkv, A_wo)
    h2 = h + _B_ref(_layernorm(h, axis=-1), B_w1, B_w2)
    return h2
```

```python
import math

import jax
import jax.numpy as jnp
from jax import lax
import jax.experimental.pallas as pl
import jax.experimental.pallas.tpu as pltpu

S, D, DFF = 2048, 640, 1536
H, DH, W = 32, 20, 256
T = 256
UNROLL = False
PV_F32 = True
EPS = 1e-5

BF, F32, U32, I32 = jnp.bfloat16, jnp.float32, jnp.uint32, jnp.int32
NN = (((1,), (0,)), ((), ()))
NT = (((1,), (1,)), ((), ()))


def _dot(a, b, dims=NN):
    return lax.dot_general(a, b, dims, preferred_element_type=F32)


def _pack(lo, hi):
    return pltpu.pack_elementwise([lo, hi], packed_dtype=BF)


def _ln(x):
    m = jnp.mean(x, axis=-1, keepdims=True)
    d = x - m
    v = jnp.mean(d * d, axis=-1, keepdims=True)
    return d * lax.rsqrt(v + EPS)


def _kernel(x_hbm, wqkv_hbm, wo_hbm, w1_hbm, w2_hbm, o_hbm,
            x_v, wqkv_v, wo_v, w1_v, w2_v, o_v,
            wvt_s, xn_s, q_s, k_s, vt_s, ot_s, h_s, hn_s, a_s,
            in_sem, x_sem, o_sem):
    NS = S // T
    HT = T // 2
    qscale = (DH ** -0.5) * math.log2(math.e)

    def x_copy(t):
        return pltpu.make_async_copy(x_hbm.at[pl.ds(t * T, T)], x_v.at[pl.ds(t * T, T)], x_sem.at[t])

    def w_copy(i):
        if i < 3:
            c = pl.ds(i * D, D)
            return pltpu.make_async_copy(wqkv_hbm.at[:, c], wqkv_v.at[:, c], in_sem.at[i])
        src, dst = ((wo_hbm, wo_v), (w1_hbm, w1_v), (w2_hbm, w2_v))[i - 3]
        return pltpu.make_async_copy(src, dst, in_sem.at[i])

    def o_copy(t, row):
        return pltpu.make_async_copy(o_v.at[pl.ds(row, T)], o_hbm.at[pl.ds(row, T)], o_sem.at[t])

    x_copy(0).start()
    w_copy(0).start()
    w_copy(1).start()
    w_copy(2).start()
    x_copy(1).start()
    for i in range(3, 6):
        w_copy(i).start()
    for t in range(2, NS):
        x_copy(t).start()

    def mult(v, n):
        return v if isinstance(v, int) else pl.multiple_of(v, n)

    lane16 = lax.broadcasted_iota(I32, (16, 128), 1)
    grp16 = lane16 >> 5
    r16 = lax.broadcasted_iota(I32, (16, 128), 0)
    i16 = lane16 & 31
    up_e = 2 * r16 > i16
    up_o = 2 * r16 + 1 > i16

    def a_ln(t):
        row = mult(t * T, T)
        xu = pltpu.bitcast(x_v[pl.ds(row, T), :], U32)
        xe = _ln(pltpu.unpack_elementwise(xu, index=0, packed_dtype=BF, unpacked_dtype=F32))
        xo = _ln(pltpu.unpack_elementwise(xu, index=1, packed_dtype=BF, unpacked_dtype=F32))
        xn_s[0:HT, :] = xe
        xn_s[HT:T, :] = xo

    def quad_tiles(tiles, lane):
        out = []
        for j in range(8):
            lo, hi = (80 * j) // 128, (80 * j + 79) // 128
            if lo == hi:
                out.append(tiles[lo])
            else:
                out.append(jnp.where(lane >= (80 * j) % 128, tiles[lo], tiles[hi]))
        return out

    def a_q(t):
        hrow = mult(t * HT, HT)
        q = _dot(xn_s[...], wqkv_v[:, 0:D]) * qscale
        qp = _pack(q[0:HT], q[HT:T])
        lane = lax.broadcasted_iota(I32, (HT, 128), 1)
        for j, qt in enumerate(quad_tiles([qp[:, 128 * c:128 * c + 128] for c in range(5)], lane)):
            q_s[j, pl.ds(hrow, HT), :] = qt

    def a_k(t):
        hrow = mult(t * HT, HT)
        k = _dot(xn_s[...], wqkv_v[:, D:2 * D])
        lane = lax.broadcasted_iota(I32, (T, 128), 1)
        for j, kt in enumerate(quad_tiles([k[:, 128 * c:128 * c + 128] for c in range(5)], lane)):
            k_s[0, j, pl.ds(hrow, HT), :] = kt[0:HT]
            k_s[1, j, pl.ds(hrow, HT), :] = kt[HT:T]

    VOFF = (0, 16, 40, 56)
    ONES = (20, 0, 20, 0)

    def a_v(t, j0, j1):
        xp = pltpu.bitcast(_pack(xn_s[0:HT, :], xn_s[HT:T, :]), BF)
        vt = _dot(pltpu.bitcast(wvt_s[40 * j0:40 * j1, :], BF), xp, NT)
        r8 = lax.broadcasted_iota(I32, (8, T), 0)
        for j in range(j0, j1):
            for h in range(4):
                b = 80 * (j - j0) + VOFF[h]
                rows = [vt[b + 8 * i:b + 8 * i + 8] for i in range(3)]
                if ONES[h]:
                    rows[2] = jnp.where(r8 >= 4, 1.0, rows[2])
                else:
                    rows[0] = jnp.where(r8 < 4, 1.0, rows[0])
                win = jnp.concatenate(rows, 0)
                for c in range(T // 128):
                    vt_s[4 * j + h, t * (T // 128) + c] = win[:, 128 * c:128 * c + 128]

    def b_qk(blk, j):
        static = isinstance(blk, int)
        z = []
        for g in range(4):
            qg = q_s[j, pl.ds(mult(blk * 64 + 16 * g, 16), 16), :]
            rows = []
            for p in range(4):
                h = (p - g) % 4
                lo = (80 * j + 20 * h) % 128
                if lo + 20 <= 128:
                    m = (lane16 >= lo) & (lane16 < lo + 20)
                else:
                    m = (lane16 >= lo) | (lane16 < lo + 20 - 128)
                rows.append(jnp.where(m, qg, jnp.uint32(0)))
            rhs = pltpu.bitcast(jnp.concatenate(rows, 0), BF)
            if static and blk < 2:
                n = 64 * blk + 16 * g + 16
                s = _dot(jnp.concatenate([k_s[0, j, 0:n, :], k_s[1, j, 0:n, :]], 0), rhs, NT)
                se = [jnp.where(up_e, -jnp.inf, s[n - 16:n])]
                so = [jnp.where(up_o, -jnp.inf, s[2 * n - 16:2 * n])]
                if n > 16:
                    se, so = [s[0:n - 16]] + se, [s[n:2 * n - 16]] + so
                se, so = jnp.concatenate(se, 0), jnp.concatenate(so, 0)
                mx = jnp.maximum(jnp.max(se, axis=0, keepdims=True), jnp.max(so, axis=0, keepdims=True))
                pp = _pack(jnp.exp2(se - mx), jnp.exp2(so - mx))
                blocks = [pp[16 * i:16 * i + 16] for i in range(n // 16)]
                z.append(blocks + [None] * (3 - g))
            else:
                rs = pl.ds(mult(blk * 64 + 16 * g - 128, 16), 144)
                s = _dot(jnp.concatenate([k_s[0, j, rs, :], k_s[1, j, rs, :]], 0), rhs, NT)
                se = jnp.concatenate([jnp.where(up_e, s[0:16], s[128:144]), s[16:128]], 0)
                so = jnp.concatenate([jnp.where(up_o, s[144:160], s[272:288]), s[160:272]], 0)
                mx = jnp.max(jnp.maximum(se, so), axis=0, keepdims=True)
                pe, po = jnp.exp2(se - mx), jnp.exp2(so - mx)
                first = _pack(jnp.where(up_e, pe[0:16], 0.0), jnp.where(up_o, po[0:16], 0.0))
                last = _pack(jnp.where(up_e, 0.0, pe[0:16]), jnp.where(up_o, 0.0, po[0:16]))
                pm = _pack(pe[16:], po[16:])
                blocks = [first] + [pm[16 * i:16 * i + 16] for i in range(7)] + [last]
                z.append([None] * g + blocks + [None] * (3 - g))
        return z

    def b_pv(blk, j, z, slot):
        static = isinstance(blk, int)
        nt = len(z[0])

        def sel(m, a, b):
            if a is None and b is None:
                return None
            zero = jnp.zeros((16, 128), U32)
            return jnp.where(m, zero if a is None else a, zero if b is None else b)

        odd, hi = (grp16 & 1) == 1, grp16 >= 2
        a = [[sel(odd, z[(i + 1) % 4][t], z[i][t]) for t in range(nt)] for i in range(4)]
        r8 = lax.broadcasted_iota(I32, (8, 128), 0)
        o = []
        for h in range(4):
            f = [sel(hi, a[(2 - h) % 4][t], a[(-h) % 4][t]) for t in range(nt)]
            f = pltpu.bitcast(jnp.concatenate(f, 0), BF)
            nk = nt // 4
            v = jnp.concatenate([vt_s[4 * j + h, blk - (nk - 1) + c] for c in range(nk)], 1)
            r = _dot(v, f)
            r = r * (1.0 / r[ONES[h]:ONES[h] + 1])
            if h:
                r = pltpu.roll(r, 128 - 32 * h, 1)
            o.append([r[0:8], r[8:16], r[16:24]])
        rows = [o[0][0], o[0][1], jnp.where(r8 < 4, o[0][2], o[1][0]), o[1][1], o[1][2],
                o[2][0], o[2][1], jnp.where(r8 < 4, o[2][2], o[3][0]), o[3][1], o[3][2]]
        ot_s[slot, 80 * j:80 * j + 80, :] = jnp.concatenate(rows, 0)

    def c_wo(t):
        row = mult(t * T, T)
        base = (t % 2) * (T // 128)
        o = jnp.concatenate([ot_s[base + c].T for c in range(T // 128)], 0)
        h = x_v[pl.ds(row, T), :].astype(F32) + _dot(o, wo_v[...])
        h_s[...] = h
        hn_s[...] = _ln(h)

    def c_ffn1(c0, c1):
        cs = slice(128 * c0, 128 * c1)
        a_s[:, cs] = jnp.maximum(_dot(hn_s[...], w1_v[:, cs]), 0.0)

    def c_ffn2(t, c0, c1):
        row = mult(t * T, T)
        cs = slice(128 * c0, 128 * c1)
        o_v[pl.ds(row, T), cs] = (h_s[:, cs] + _dot(a_s[...], w2_v[:, cs])).astype(BF)

    def step(ta, tb, tc):
        dense = []
        if tc is not None:
            dense.append((5, lambda: c_wo(tc)))
        if ta is not None:
            a_ln(ta)
            dense.append((5, lambda: a_q(ta)))
            dense.append((5, lambda: a_k(ta)))
            dense.append((2.5, lambda: a_v(ta, 0, 4)))
            dense.append((2.5, lambda: a_v(ta, 4, 8)))
        if tc is not None:
            for c in range(0, 12, 3):
                dense.append((3, lambda c=c: c_ffn1(c, c + 3)))
            for c in range(5):
                dense.append((2.4, lambda c=c: c_ffn2(tc, c, c + 1)))
        if tb is None:
            for _, f in dense:
                f()
            return
        units = [(b, j) for b in range(T // 128) for j in range(8)]
        total = sum(w for w, _ in dense)
        done, di = 0.0, 0
        pending = None
        for u, (b, j) in enumerate(units):
            blk = tb * (T // 128) + b
            z = b_qk(blk, j)
            if pending is not None:
                b_pv(*pending)
            pending = (blk, j, z, (tb % 2) * (T // 128) + b)
            target = total * (u + 1) / (len(units) + 1)
            while di < len(dense) - 1 and done + dense[di][0] / 2 <= target:
                done += dense[di][0]
                dense[di][1]()
                di += 1
        b_pv(*pending)
        for _, f in dense[di:]:
            f()

    x_copy(0).wait()
    a_ln(0)
    w_copy(0).wait()
    a_q(0)
    w_copy(1).wait()
    a_k(0)
    w_copy(2).wait()
    wvt_s[...] = pltpu.bitcast(wqkv_v[:, 2 * D:3 * D].T, U32)
    a_v(0, 0, 8)
    x_copy(1).wait()
    step(1, 0, None)
    for i in range(3, 6):
        w_copy(i).wait()

    def body(t):
        x_copy(t + 1).wait()
        step(t + 1, t, t - 1)
        o_copy(t - 1, mult((t - 1) * T, T)).start()

    if UNROLL:
        for t in range(1, NS - 1):
            body(t)
    else:
        pl.loop(1, NS - 1)(body)
    step(None, NS - 1, NS - 2)
    o_copy(NS - 2, (NS - 2) * T).start()
    step(None, None, NS - 1)
    o_copy(NS - 1, (NS - 1) * T).start()
    for t in range(NS):
        o_copy(t, t * T).wait()


@jax.jit
def pallas_sequential_preLN__sliding_block__dense_activation_relu__prompt_kernel(
    A_x, A_wqkv, A_wo, B_x, B_w1, B_w2,
):
    del B_x
    hbm = pl.BlockSpec(memory_space=pltpu.HBM)
    ns = S // T
    out = pl.pallas_call(
        _kernel,
        out_shape=jax.ShapeDtypeStruct((S, D), BF),
        in_specs=[hbm] * 5,
        out_specs=hbm,
        scratch_shapes=[
            pltpu.VMEM((S, D), BF), pltpu.VMEM((D, 3 * D), BF), pltpu.VMEM((D, D), BF),
            pltpu.VMEM((D, DFF), BF), pltpu.VMEM((DFF, D), BF), pltpu.VMEM((S, D), BF),
            pltpu.VMEM((D // 2, D), U32),
            pltpu.VMEM((T, D), F32),
            pltpu.VMEM((8, S // 2, 128), U32),
            pltpu.VMEM((2, 8, S // 2, 128), F32),
            pltpu.VMEM((H, S // 128, 24, 128), F32),
            pltpu.VMEM((2 * T // 128, D, 128), F32),
            pltpu.VMEM((T, D), F32), pltpu.VMEM((T, D), F32), pltpu.VMEM((T, DFF), F32),
            pltpu.SemaphoreType.DMA((6,)), pltpu.SemaphoreType.DMA((ns,)), pltpu.SemaphoreType.DMA((ns,)),
        ],
        compiler_params=pltpu.CompilerParams(vmem_limit_bytes=100 * 1024 * 1024),
        name="fused_block",
    )(A_x.reshape(S, D), A_wqkv, A_wo, B_w1, B_w2)
    return out.reshape(1, S, D)
```

```python
import functools
import itertools
import math

import jax
import jax.numpy as jnp
from jax import lax
import jax.experimental.pallas as pl
import jax.experimental.pallas.tpu as pltpu

S, D, DFF = 2048, 640, 1536
H, DH = 32, 20
EPS = 1e-5
T = 256
HT = T // 2
PR = HT // 2
NS = S // T
RANGE = 2.0 ** 60

SCHEDULE = dict(
    head=1, tail=3,
    lag=0, gap=2,
    queries=34,
    margin=1,
    hold=8,
    dither=0)
SCHEDULE_0 = dict(marks=(0, 2, 3, 4, 6, 8, 10, 12, 13), lag=2, gap=0, queries=math.inf, dither=17)
SCHEDULE_1 = dict(dither=24)
SCHEDULE_LOOP = dict(dither=5)
SCHEDULE_END = dict(head=2, tail=0, margin=2, hold=12, dither=18)
SLOT_O = (2, 0, 3, 1, 6, 4, 7, 5)
SLOT_A = (1, 0, 3, 2, 5, 4, 7, 6)
PLACE_X = (1, 3, 0, 2, 5, 7, 4, 6)

BF, F32, U32, I32 = jnp.bfloat16, jnp.float32, jnp.uint32, jnp.int32
NN = (((1,), (0,)), ((), ()))
NT = (((1,), (1,)), ((), ()))


def _dot(a, b, dims=NN):
    return lax.dot_general(a, b, dims, preferred_element_type=F32)


def _pack(lo, hi):
    return pltpu.pack_elementwise([lo, hi], packed_dtype=BF)


def _part(u, index):
    return pltpu.unpack_elementwise(u, index=index, packed_dtype=BF, unpacked_dtype=F32)


def _unpack(u):
    return jnp.concatenate([_part(u, 0), _part(u, 1)], 0)


def _repack(v):
    n = v.shape[0] // 2
    return _pack(v[:n], v[n:])


def _bf(u):
    return pltpu.bitcast(u, BF)


def _normed(x):
    d = x - jnp.mean(x, axis=-1, keepdims=True)
    return d * lax.rsqrt(jnp.mean(d * d, axis=-1, keepdims=True) + EPS)


def _drain(gen):
    for _ in gen:
        pass


class _Scheme:
    def __init__(self, t, alpha, rounds, groups):
        self.t = t
        self.alpha = alpha
        self.pairs = [r[:2] for r in rounds]
        self.order = [k for i, j, c, d in rounds for k in (("g", i, j), ("g", j, i), ("m", i, j), (c, d, d))]
        last = {i: n for n, pair in enumerate(self.pairs) for i in pair}
        self.done = [[i for i in sorted(last) if last[i] == n] for n in range(len(rounds))]
        self.groups = [[k for k in self.order if (k[1] in singles if k[0] in "pq" else tuple(sorted(k[1:])) in pairs)]
                       for pairs, singles in groups]
        assert sorted(sum(self.groups, [])) == sorted(self.order)

    def shear(self, x1, x2, j, sign=-1):
        t = sign * self.t[j]
        v = x1 if abs(t) <= 1 else x1 * float(abs(t))
        return x2 if t == 0 else x2 + v if t > 0 else x2 - v

    def left(self, x1, y, keys):
        out = {}
        for kind, i, j in keys:
            if kind in "pq":
                out[kind, i, j] = (x1 if kind == "p" else y)[i]
            elif kind == "m":
                m = out["m", i, j] = y[i] + y[j]
                for a, b in ((i, j), (j, i)):
                    c = self.t[b] - self.t[a]
                    v = x1[b] if abs(c) == 1 else x1[b] * float(abs(c))
                    out["g", a, b] = m + v if c > 0 else m - v
        return out

    def update(self, acc, r):
        def add(key, v, sign=1):
            if key not in acc:
                acc[key] = (sign, v)
            else:
                s, old = acc[key]
                acc[key] = (s, old + v) if s == sign else (1, old - v if s > 0 else v - old)

        (_, i, j), _, _, single = r
        add(single[:2], r[single])
        delta = self.t[i] - self.t[j]
        c = r["m", i, j] - r["g", i, j] - r["g", j, i]
        if abs(delta) != 1:
            c = c * (1.0 / abs(delta))
        add(("p", i), c, 1 if delta > 0 else -1)
        add(("p", j), c, -1 if delta > 0 else 1)
        add(("q", i), r["g", i, j])
        add(("q", j), r["g", j, i])

    def result(self, acc, i):
        (s1, y1), (s2, z) = acc["p", i], acc["q", i]
        assert s1 == s2 == 1
        return y1, self.shear(y1, z, i, 1)


SQUARE = _Scheme(
    (0, 1, -1, 2, -2), 0.625,
    ((0, 1, "p", 0), (0, 2, "q", 0), (0, 3, "p", 3), (0, 4, "p", 4), (1, 2, "p", 1),
     (1, 3, "q", 1), (1, 4, "q", 4), (2, 3, "p", 2), (2, 4, "q", 2), (3, 4, "q", 3)),
    ((((0, 1), (0, 2), (1, 2)), (0,)), (((0, 3), (0, 4), (3, 4)), (3,)),
     (((1, 3), (1, 4)), (1, 4)), (((2, 3), (2, 4)), (2,))))
BAND = _Scheme(
    (0, 1, -1, 0, 1, -1), 1.0,
    ((0, 5, "p", 5), (1, 5, "q", 5), (3, 5, "p", 3), (4, 5, "p", 4), (0, 1, "p", 0), (0, 2, "q", 0),
     (0, 4, "q", 4), (1, 2, "p", 1), (1, 3, "q", 1), (2, 4, "p", 2), (3, 4, "q", 3), (2, 3, "q", 2)),
    ((((0, 1), (0, 5), (1, 5)), (0, 5)), (((3, 4), (3, 5), (4, 5)), (3,)),
     (((0, 2), (0, 4), (2, 4)), (2, 4)), (((1, 2), (1, 3), (2, 3)), (1,))))
ALL = tuple(range(5))


NORM_COST = [(40, 9)] * 4 + [(60, 5)] * 8 + [(83, 21)] * 8


def _place(fore, work):
    n = len(fore)
    base = [0.0] + list(itertools.accumulate(fore))
    sums = [(a, z, sum(c for _, c in pieces)) for a, z, pieces in work]
    low = [base[t] + sum(c for a, z, c in sums if z <= t) for t in range(n + 1)]
    high = [base[t] + sum(c for a, z, c in sums if a < t) for t in range(n + 1)]
    level, t = [0.0], 0
    while t < n:
        up, dn, tu, td = math.inf, -math.inf, t, t
        end, slope = n, (low[n] - level[t]) / (n - t)
        for e in range(t + 1, n + 1):
            su, sd = (high[e] - level[t]) / (e - t), (low[e] - level[t]) / (e - t)
            if su < dn - 1e-9:
                end, slope = td, dn
                break
            if sd > up + 1e-9:
                end, slope = tu, up
                break
            if su <= up:
                up, tu = su, e
            if sd >= dn:
                dn, td = sd, e
        level += [level[t] + slope * k for k in range(1, end - t + 1)]
        t = end
    queues = []
    for (a, z, pieces), (_, _, total) in zip(work, sums):
        cum = [0.0] + list(itertools.accumulate(c for _, c in pieces))
        queues.append([(a + (z - a) * (lo + c / 2) / total, a, z, item, c)
                       for lo, (item, c) in zip(cum, pieces)])
    done, out = 0.0, []
    for t in range(n):
        while True:
            ready = [q for q in queues if q and q[0][1] <= t]
            if not ready:
                break
            late = [q for q in ready if q[0][2] <= t + 1]
            q = min(late or ready, key=lambda q: q[0][0])
            if not late and base[t + 1] + done + q[0][4] / 2 > level[t + 1]:
                break
            done += q[0][4]
            out.append((t, q.pop(0)[3]))
    return out


def _kernel(x_hbm, wqkv_hbm, wo_hbm, w1_hbm, w2_hbm, o_hbm,
            wq_s, wk_s, wv_s, wo_s, w1_s, w2_s, x_s, x2_s, o_s, h_s, a_s, b_s,
            mask_s, range_s, q_s, k_s, v_s, vt_s, ot_s, out_s, s_s, qkv_s,
            w_sem, x_sem, o_sem, idle_sem):
    F = len(BAND.order) * PR
    weights = {"q": wq_s, "k": wk_s, "v": wv_s, "o": wo_s, "w1": w1_s, "w2": w2_s}
    zero = pl.semaphore_read(idle_sem)
    hold = [SCHEDULE["hold"]]
    prepared, building = [], []
    written = []

    def rows(start, n, multiple=8):
        return pl.ds(start if isinstance(start, int) else pl.multiple_of(start, multiple), n)

    def get(buf, start, n):
        return pltpu.bitcast(buf[rows(start, n), :], F32)

    def put(buf, start, v):
        buf[rows(start, v.shape[0]), :] = v if v.dtype == U32 else pltpu.bitcast(v, U32)

    def tick(buf, v):
        buf[rows(zero + (buf.shape[0] - 8), 8), 0:128] = pltpu.bitcast(v, U32)

    def x_copies(t):
        n = HT if t < 3 else (NS - 3) * HT
        return [pltpu.make_async_copy(x_hbm.bitcast(U32).at[pl.ds(t * HT, n), pl.ds(128 * c, 128)],
                                      x_s.at[pl.ds(F + 5 * T + c * (S // 2) + t * HT, n)], x_sem.at[t])
                for c in ALL]

    def w_copies(name, c=0, tiles=None):
        i = list(weights).index(name)
        src = (wqkv_hbm, wqkv_hbm, wqkv_hbm, wo_hbm, w1_hbm, w2_hbm)[i]
        n = 128 * (tiles or weights[name].shape[1] // 128 - c)
        return [pltpu.make_async_copy(src.bitcast(U32).at[:, pl.ds((i * D if i < 3 else 0) + 128 * c, n)],
                                      weights[name].at[pl.ds(0, src.shape[0] // 2), pl.ds(128 * c, n)],
                                      w_sem.at[6 if c else i])]

    def o_copy(t, n, c):
        where = (pl.ds(t * T, n * T), pl.ds(128 * c, 128))
        return pltpu.make_async_copy(out_s.at[where], o_hbm.at[where], o_sem)

    def start(*copies):
        for copy in itertools.chain(*copies):
            copy.start()

    def wait(*copies):
        for copy in itertools.chain(*copies):
            copy.wait()

    def x_words(t, c, r, n):
        return x_s[rows(F + 5 * T + c * (S // 2) + t * HT + r, n), :]

    lane8 = lax.broadcasted_iota(I32, (8, 128), 1)
    row8 = lax.broadcasted_iota(I32, (8, 128), 0)

    def key_later(r0, parity):
        r, c = row8 + r0, lane8
        return 16 * (r & 1) + 2 * (r >> 1) + parity > (c & 1) + 8 * (c & 2) + (((c & 31) >> 2) << 1)

    later = [[key_later(8 * u, p) for p in range(2)] for u in range(2)]
    bit = [(lane8 >> n) & 1 for n in range(7)]
    source = [bit[4] + 2 * bit[2] + 4 * bit[3] + 8 * bit[0] + 16 * bit[1] + 32 * ((bit[5] + 2 * bit[6] + h) & 3)
              for h in range(4)]

    def tables():
        range_s[...] = jnp.ones(range_s.shape, F32)
        for head in range(H):
            mask_s[32 + head] = jnp.where(((lane8 - DH * head) & 127) < DH, jnp.uint32(0xFFFFFFFF), jnp.uint32(0))
        for h in range(4):
            group = ((lane8 >> 5) - h) & 3
            for t in range(8):
                old = [(group < t // 2) | ((group == t // 2) & later[t % 2][p]) for p in range(2)]
                mask_s[8 * h + t] = (jnp.where(old[0], jnp.uint32(0xFFFF), jnp.uint32(0))
                                     | jnp.where(old[1], jnp.uint32(0xFFFF0000), jnp.uint32(0)))

    def block(k, n, r=0, size=64):
        return (slice(64 * k + r, 64 * k + r + size), slice(128 * n, 128 * n + 128))

    def terms(name, n, i, j):
        if name in "qkvo":
            return [(1, (j, i))]
        own, other = (i, j) if name == "w1" else (j, i)
        at = [(k, 6 * n + own) if name == "w1" else (6 * n + own, k) for k in ALL]
        far = (own + 3) % 6
        return [(1, at[other])] if far == 5 else [(2, at[far])] if other == 5 else [(1, at[other]), (-1, at[far])]

    def position(name, n, key):
        def raw(kind, i, j):
            return kind == "g" and [c for c, _ in terms(name, n, i, j)] == [1]

        if raw(*key):
            return terms(name, n, *key[1:])[0][1]
        kept = [k for k in (SQUARE if name in "qkvo" else BAND).order if not raw(*k)]
        k, c = divmod(n * len(kept) + kept.index(key), weights[name].shape[1] // 128)
        return k + (12 if name == "w2" else 5), c

    def right(name, n, key):
        assert prepared.count((name, n)) == 8
        return _bf(weights[name][block(*position(name, n, key))])

    def prepare(name, n=0, part=range(8)):
        buf, scheme = weights[name], SQUARE if name in "qkvo" else BAND

        def stream():
            for r in [8 * e for e in part]:
                def load(i, j):
                    (c, v), *rest = [(c, _unpack(buf[block(*at, r, 8)])) for c, at in terms(name, n, i, j)]
                    return v - rest[0][1] if rest else v + v if c == 2 else v

                def store(key, v):
                    at = position(name, n, key)
                    if at[0] >= (12 if name == "w2" else 5):
                        buf[block(*at, r, 8)] = _repack(v)

                acc = {}
                for i in range(len(scheme.t)):
                    acc["p", i] = acc["q", i] = load(i, i)
                for e, (i, j) in enumerate(scheme.pairs):
                    if e % 4 == 2:
                        yield
                    wij, wji = load(i, j), load(j, i)
                    for key, v in ((("g", i, j), wij), (("g", j, i), wji), (("m", i, j), wij + wji)):
                        store(key, v)
                    acc["p", j], acc["p", i] = acc["p", j] + wij, acc["p", i] + wji
                    acc["q", i], acc["q", j] = acc["q", i] - wij, acc["q", j] - wji
                for (kind, i), v in acc.items():
                    store((kind, i, i), v)
                prepared.append((name, n))
                yield

        costs = [(42, 3), (60, 5), (70, 25)] if scheme is SQUARE else [(80, 7), (95, 12), (95, 12), (60, 30)]
        return [(buf, stream(), costs * len(part))]

    def slots(buf):
        if any(buf is other for other in (x_s, x2_s)):
            return range(8)
        return SLOT_O if buf is o_s or buf is h_s else SLOT_A

    def blocks(buf, base, place=range(8)):
        return lambda c, half, r: get(buf, base + c * T + half * HT + 16 * place[r // 16], 16)

    def operands(scheme, buf, load):
        def stream():
            held = []
            building.append(buf)
            for r in range(0, HT, 16):
                for keys in scheme.groups:
                    idx = sorted({i for k in keys for i in k[1:]})
                    x1, y = [{c: load(c, half, r) for c in idx} for half in range(2)]
                    held += [(scheme.order.index(k) * PR + 8 * slots(buf)[r // 16], _repack(v))
                             for k, v in scheme.left(x1, y, keys).items()]
                    while len(held) > hold[0]:
                        put(buf, *held.pop(0))
                    yield
            for row, u in held:
                put(buf, row, u)
            building.pop()
        return buf, stream(), [(3.3 * len(keys), len(keys) + 1) for keys in scheme.groups] * 8

    def layer_norm(scheme, load, buf, place, shuffled=None):
        mean, var, scale = {}, {}, {}
        for r in range(0, HT, 16):
            for half in range(2):
                x = [load(c, half, r) for c in ALL]
                mean[half, r] = jnp.sum(x[0] + x[1] + x[2] + x[3] + x[4], axis=1, keepdims=True) * (1.0 / D)
            if r % 32:
                yield
        for r in range(0, HT, 16):
            for half in range(2):
                d = [load(c, half, r) - mean[half, r] for c in ALL]
                d = [v * v for v in d]
                var[half, r] = jnp.sum(d[0] + d[1] + d[2] + d[3] + d[4], axis=1, keepdims=True) * (1.0 / D)
            if r + 16 < HT:
                yield

        def scales(r):
            for half in range(2):
                s = lax.rsqrt(var[half, r] + EPS)
                scale[half, r] = s if half or scheme.alpha == 1.0 else s * scheme.alpha
                for c, v in ((-2, mean[half, r]), (-1, scale[half, r])) if shuffled else ():
                    put(buf, h_row(0, c) + half * HT + r, jnp.broadcast_to(v, (16, 128)))

        ahead = 32 if shuffled else 16
        for r in range(0, ahead, 16):
            scales(r)
        yield
        for r in range(0, HT, 16):
            y = []
            for half in range(2):
                m, s = [shuffled(c, half, r) for c in (-2, -1)] if shuffled else (mean[half, r], scale[half, r])
                y.append([((shuffled or load)(c, half, r) - m) * s for c in ALL])
                if scheme is BAND:
                    y[half].append((y[half][0] + y[half][1] + y[half][2] + y[half][3] + y[half][4]) * 0.5)
            if r + ahead < HT:
                scales(r + ahead)
            for c, (y1, y2) in enumerate(zip(*y)):
                put(buf, F + c * T + 16 * place[r // 16], y1)
                put(buf, F + c * T + HT + 16 * place[r // 16], scheme.shear(y1, y2, c))
            yield

    def x_operands(t, buf):
        def load(c, half, r):
            return _part(x_words(t, c, half * PR + 16 * (r // 32), 16), (r // 16) % 2)
        return [(x_s, layer_norm(SQUARE, load, buf, PLACE_X), [(alu + 20, st) for alu, st in NORM_COST]),
                operands(SQUARE, buf, blocks(buf, F, PLACE_X))]

    def h_row(slot, c):
        return F + (8 + (5 * slot if c >= 0 else 0) + c) * T + 16

    def h_operands(slot=0):
        def shuffled(c, half, r):
            row = h_row(slot, c) + half * HT + 32 * (r // 32) + (r // 16) % 2
            return pltpu.bitcast(jnp.concatenate([h_s[pl.ds(row + p, 8, stride=4), :] for p in (0, 2)], 0), F32)
        return [(h_s, layer_norm(BAND, blocks(h_s, h_row(slot, 0)), h_s, range(8), shuffled), NORM_COST),
                operands(BAND, h_s, blocks(h_s, F))]

    def o_operands():
        def load(*where):
            assert len(written) == 10, "the attention output of the next tile is already arriving"
            return blocks(o_s, F)(*where)
        return [operands(SQUARE, o_s, load)]

    def a_operands(buf):
        def load(c, half, r):
            row = F + c * T + half * HT + 32 * (r // 32) + 8 * ((r // 16) % 2)
            return jnp.concatenate([get(buf, row + p, 8) for p in (0, 16)], 0)

        return [operands(BAND, buf, load)]

    def left(buf, n):
        assert not any(buf is other for other in building)
        return _bf(jnp.concatenate([buf[rows(n * PR + 8 * k, 8), :] for k in slots(buf)], 0))

    def product(scheme, passes, finish, alu, stores):
        def gen():
            acc, jobs = {}, 0
            for parts in passes:
                r = {}
                for e, k in enumerate(scheme.order):
                    for buf, name, n in parts:
                        y = _dot(left(buf, e), right(name, n, k))
                        r[k] = r[k] + y if k in r else y
                        jobs += 1
                        if e % 4 == 3 and jobs % (4 * len(parts)) == 0:
                            scheme.update(acc, r)
                            r = {}
                            for i in scheme.done[e // 4] if parts is passes[-1] else ():
                                finish(i, *scheme.result(acc, i))
                        if jobs % 4 == 0:
                            yield y

        load = []
        for parts in passes:
            for done in scheme.done:
                d = len(done) if parts is passes[-1] else 0
                load += [(16, 32, 32)] * (len(parts) - 1)
                load += [(16, 74 + 32 * len(parts) + (20 + alu) * d, 64 + (stores - 32) * d)]
        return gen(), load

    def quad(tiles, j):
        lo, hi = (80 * j) // 128, (80 * j + 79) // 128
        if lo == hi:
            return tiles[lo]
        lane = lax.broadcasted_iota(I32, tiles[lo].shape, 1)
        return jnp.where(lane >= (80 * j) % 128, tiles[lo], tiles[hi])

    def qkv_finish(t, name, scale):
        tiles = {}
        both = (DH ** -0.5) * math.log2(math.e) if name == "q" else 1.0

        def finish(c, y1, y2):
            y = jnp.concatenate([v if s == 1.0 else v * s for v, s in ((y1, scale * both), (y2, both))], 0)
            if name != "k":
                y = jnp.concatenate([_repack(y[r:r + 32]) for r in range(0, T, 32)], 0)
            tiles[c] = y
            if name == "v":
                put(v_s, c * HT, y)
                return
            for j in range(8):
                if (80 * j + 79) // 128 == c:
                    put(q_s if name == "q" else k_s, (j * NS + t) * y.shape[0], quad(tiles, j))
        return finish

    def project(t, name, buf=x_s):
        cost = {"q": (60, 26), "k": (42, 52), "v": (32, 16)}[name]
        return product(SQUARE, [[(buf, name, 0)]], qkv_finish(t, name, 1.0 / SQUARE.alpha), *cost)

    def project_raw(xn, name):
        n = xn.shape[0]

        def gen():
            finish, buf = [qkv_finish(t, name, 1.0) for t in range(n // T)], weights[name]
            for c in ALL:
                w = _bf(buf[0:D // 2, 128 * c:128 * c + 128])
                y = _dot(xn[:, 0:512], w[0:512]) + jnp.concatenate(
                    [_dot(xn[r:r + n // 4, 512:D], w[512:D]) for r in range(0, n, n // 4)], 0)
                for t, f in enumerate(finish):
                    f(c, y[t * T:t * T + HT], y[t * T + HT:t * T + T])
                yield y
        return gen(), [(n // 8, 170, 55)] * 5

    FIRST = (0, 16, 40, 56)
    ONES = (20, 0, 20, 0)

    def vt_rows(head, blk):
        return rows((head * (S // 128) + blk) * 32, 24)

    def v_transpose(t):
        def stream():
            for b in range(2):
                tiles = {}
                for c in ALL:
                    vt = _bf(v_s[rows(c * HT + 64 * b, 64), :]).T.astype(F32)
                    tiles.update({16 * c + i: vt[8 * i:8 * i + 8] for i in range(16)})
                    for head in range(H):
                        first = (80 * (head // 4) + FIRST[head % 4]) // 8
                        if (first + 2) // 16 == c:
                            v = [tiles[first + i] for i in range(3)]
                            if ONES[head % 4]:
                                v[2] = jnp.where(row8 >= 4, 1.0, v[2])
                            else:
                                v[0] = jnp.where(row8 < 4, 1.0, v[0])
                            vt_s[vt_rows(head, 2 * t + b), :] = jnp.concatenate(v, 0)
                    yield
        return [(v_s, stream(), [(24, 20)] * 10)]

    def out_proj(t, slot=0):
        def finish(c, y1, y2):
            x = jnp.concatenate([_unpack(x_words(t, c, r, 16)) for r in range(0, HT, 16)], 0)
            put(h_s, h_row(slot, c), x + jnp.concatenate([y1 * (1.0 / SQUARE.alpha), y2], 0))
        return product(SQUARE, [[(o_s, "o", 0)]], finish, 80, 32)

    def ffn1(bufs, n):
        def finish(c, y1, y2):
            y1, y2 = jnp.maximum(y1, 0.0), jnp.maximum(y2, 0.0)
            put(bufs[n], F + c * T, jnp.concatenate([y1, BAND.shear(y1, y2, c)], 0))
        return product(BAND, [[(h_s, "w1", n)]], finish, 44, 32)

    def ffn2(t, bufs, slot=0, passes=((0, 1),), stored=None):
        shared = []

        def finish(c, y1, y2):
            y = jnp.concatenate([y1, y2], 0)
            if c == 5:
                shared.append(y * 0.5)
                return
            y = y + shared[0] + get(h_s, h_row(slot, c), T)
            out_s[rows(t * T, T, T), 128 * c:128 * c + 128] = _bf(jnp.concatenate(
                [_repack(y[p:p + 32]) for p in range(0, T, 32)], 0))
            if stored is not None:
                stored(c)
        return product(BAND, [[(bufs[n], "w2", n) for n in parts] for parts in passes], finish, 110, 32)

    def scores(blk, j, buf):
        start_up = isinstance(blk, int) and blk < 2
        slabs = [t ^ 7 for t in range(8 * (blk + 1) if start_up else 16)]
        first = j * S + (0 if start_up else blk * 128 - 256)
        probs = {}
        for g in range(3, -1, -1) if start_up and j % 2 else range(4):
            q = q_s[rows(j * (S // 2) + blk * 64 + 16 * g, 16), :]
            heads = [q[r:r + 8] & mask_s[32 + 4 * j + (p - g) % 4] for p in range(4) for r in (0, 8)]
            if start_up:
                keys = [t for t in slabs if t < 8 * blk + 2 * g + 2]
            else:
                keys = [k for t in slabs for k in ([t] if t >= 2 * g else []) + ([t + 16] if t < 2 * g + 2 else [])]
            s = _dot(jnp.concatenate([get(k_s, first + 32 * (k // 2) + 8 * (k % 2) + 16 * p, 8)
                                      for k in keys for p in range(2)], 0), _bf(jnp.concatenate(heads, 0)), NT)
            found = {k: (s[16 * n:16 * n + 8], s[16 * n + 8:16 * n + 16]) for n, k in enumerate(keys)}
            for t in slabs:
                v = found.get(t, found.get(t + 16))
                if start_up and t // 2 == 4 * blk + g:
                    v = [jnp.where(later[t % 2][p], -jnp.inf, v[p]) for p in range(2)]
                elif t in found and t + 16 in found:
                    v = [jnp.where(later[t % 2][p], v[p], found[t + 16][p]) for p in range(2)]
                probs[g, t] = None if v is None else _pack(jnp.exp2(v[0]), jnp.exp2(v[1]))
            if g == 3:
                last = s

        def select(pick, a, b):
            if a is None and b is None:
                return None
            nil = jnp.zeros((8, 128), U32)
            return jnp.where(pick, nil if a is None else a, nil if b is None else b)

        out = {}
        for t in slabs:
            z = [select((lane8 & 32) != 0, probs[(i + 1) % 4, t], probs[i, t]) for i in range(4)]
            for h in range(4):
                f = out[h, t] = select(lane8 >= 64, z[(2 - h) % 4], z[(-h) % 4])
                if t < 8 and not start_up:
                    out[h, t] = f & mask_s[8 * h + t]
                    out[h, t + 16] = f ^ out[h, t]
        for (h, t), f in out.items():
            put(buf, 208 * h + 8 * t, f)
        return last

    def mix(t, b, j, buf):
        blk = 2 * t + b
        n = min(blk + 1, 3) if isinstance(blk, int) else 3
        raw = [_dot(jnp.concatenate([vt_s[vt_rows(4 * j + h, blk - (n - 1) + c), :] for c in range(n)], 1),
                    _bf(buf[rows(208 * h, 64 * n), :])) for h in range(4)]
        yield
        o, sums, scale = [], [], 1.0 if b else SQUARE.alpha
        for h, r in enumerate(raw):
            total = r[ONES[h]:ONES[h] + 1]
            sums.append(total)
            inv = pltpu.reciprocal(total, approx=True)
            r = r * (inv * (2.0 * scale - (total * scale) * inv))
            o.append([jnp.take_along_axis(r[p:p + 8], source[h], 1) for p in (0, 8, 16)])
        range_s[0:1, :] = functools.reduce(jnp.minimum, sums, range_s[0:1, :])
        range_s[8:9, :] = functools.reduce(jnp.maximum, sums, range_s[8:9, :])
        ot_s[b, 80 * j:80 * j + 80, :] = jnp.concatenate(
            [v for h in (0, 2) for v in (o[h][0], o[h][1], jnp.where(row8 < 4, o[h][2], o[h + 1][0]),
                                         o[h + 1][1], o[h + 1][2])], 0)
        for c in range((80 * j) // 128, (80 * j + 80) // 128):
            y, home = ot_s[b, 128 * c:128 * c + 128, :].T, F + c * T
            written[:] = (written if len(written) < 10 else []) + [c]
            put(o_s, home + HT * b, SQUARE.shear(get(o_s, home, HT), y, c) if b else y)

    def step(t, stages, tuning, after=0, more=False):
        cfg = {**SCHEDULE, **tuning}
        hold[0] = cfg["hold"]
        first = isinstance(t, int) and t == 0
        units, lag = 0 if t is None else 16, cfg["lag"]
        total = sum(n for _, n, _ in stages)
        marks = [0]
        if first:
            marks = [r for r in cfg["marks"] for _ in range(2)][:units + 1]
        elif units:
            span = total - after - cfg["tail"]
            marks = [cfg["head"] + ((span - cfg["head"]) * u) // units for u in range(units + 1)]
        order = [(r, 99, "dense", r) for r in range(total)]
        for u in range(units):
            order.append((marks[u], u | first, "scores", u))
            order.append((marks[min(u + lag, units)] + cfg["gap"], ((u + lag) | first) + 0.5, "mix", u))
        prog = [e[2:] for e in sorted(order, key=lambda e: e[:2])]
        assert all(prog.index(("mix", u)) < prog.index(("scores", u + len(s_s))) for u in range(units - len(s_s)))

        def cost(alu, stores):
            return alu / 4 + stores

        loads = [product[1].pop(0) for product, n, _ in stages for _ in range(n)]
        fore, clock, due = [], {}, 0
        for key in prog:
            clock[key] = len(fore)
            kind, u = key
            if kind == "dense":
                fore += [(key, r, (cost(*loads[u][1:]) + due) / loads[u][0]) for r in range(loads[u][0])]
                due = 0
            elif kind == "scores":
                fore += [(key, r, cost(13, 3)) for r in range(16 * (u // 8) + 10 if first else 36)]
            else:
                due = cost(60, 10) + ((80 * (u % 8) + 80) // 128 - (80 * (u % 8)) // 128) * cost(16, 16)

        work, begin = [], 0
        for i, (_, n, streams) in enumerate(stages):
            if streams:
                end = begin + n + sum(s[1] for s in itertools.takewhile(lambda s: s[2] is None, stages[i + 1:]))
                work.append((clock["dense", begin], clock.get(("dense", end - cfg["margin"]), len(fore)),
                             [((buf, g), cost(*c)) for buf, g, costs in streams for c in costs]))
            begin += n
        plan = {key: [] for key in prog}
        wobble = [6 * ((n + 1) * cfg["dither"] * 0.6180339887 % 1.0) for n in range(len(fore) + 1)]
        for n, item in _place([c + wobble[n + 1] - wobble[n] for n, (_, _, c) in enumerate(fore)], work):
            plan[fore[n][0]].append((fore[n][1], item))
        for u in range(units):
            if clock["scores", u] >= cfg["queries"]:
                key, r, _ = fore[clock["scores", u] - cfg["queries"]]
                plan[key].append((r, (q_s, None)))

        def rounds():
            running = ()
            for i, (product, n, streams) in enumerate(stages):
                if streams is not None:
                    for _, g, _ in running:
                        _drain(g)
                    running = streams
                for _ in range(n):
                    yield next(product[0])
                if not more and not any(s[0] is product for s in stages[i + 1:]):
                    _drain(product[0])
            for _, g, _ in running:
                _drain(g)

        dense, mixing = rounds(), ()
        for key in prog:
            kind, u = key
            if kind == "mix":
                _drain(mixing)
                mixing = mix(t, *divmod(u, 8), s_s[u % len(s_s)])
                next(mixing)
                continue
            if kind == "dense":
                y = next(dense)
            else:
                y = scores(2 * t + u // 8, u % 8, s_s[u % len(s_s)])
            for r, (buf, g) in sorted(plan[key], key=lambda e: e[0]):
                r = min(8 * r, y.shape[0] - 8)
                tick(buf, y[r:r + 8])
                if g is not None:
                    next(g)
            if kind == "dense":
                _drain(mixing)
        _drain(mixing)
        _drain(dense)

    def arrival(name):
        def stream():
            wait(w_copies(name))
            yield
        return [(v_s, stream(), [(1, 1)])]

    def run(streams):
        for _, g, _ in streams:
            _drain(g)

    def prologue():
        start(x_copies(0), x_copies(1), w_copies("k", 0, 2))
        tables()
        xn = []
        for t in range(2):
            wait(x_copies(t))
            if t == 1:
                start(w_copies("k", 2))
            y = _normed(_unpack(jnp.concatenate([x_words(t, c, 0, HT) for c in ALL], 1)))
            xn += [_repack(y[p + r:p + r + 16]) for r in range(0, HT, 16) for p in (0, HT)]
        xn = _bf(jnp.concatenate(xn, 0))
        run(x_operands(1, x_s))
        wait(w_copies("k", 0, 2))
        start(w_copies("v"))
        k, _ = project_raw(xn, "k")
        next(k), next(k)
        wait(w_copies("k", 2))
        start(w_copies("q"), x_copies(2))
        _drain(k)
        wait(w_copies("v"))
        step(None, [(project_raw(xn[0:T], "v"), 5, prepare("k"))], {})
        run(prepare("v"))
        v = project(1, "v")
        step(None, [(v, 3, v_transpose(0)), (v, 2, ())], {"margin": 0}, more=True)
        wait(w_copies("q"), x_copies(2))
        start(w_copies("o"), w_copies("w1"), w_copies("w2"))
        step(None, [(project_raw(xn[0:T], "q"), 5, x_operands(2, x2_s))], {})
        step(0, [(v, 5, prepare("q")), (project(1, "q"), 10, v_transpose(1))], SCHEDULE_0)
        wait(w_copies("o"), w_copies("w1"))
        start(x_copies(3))
        q, (norm, sums) = project(2, "q", x2_s), h_operands()
        step(1, [(project(2, "k", x2_s), 10, o_operands() + prepare("o") + prepare("w1", 0, range(3))),
                 (out_proj(0), 10, prepare("w1", 0, range(3, 8)) + prepare("w1", 1, range(5))),
                 (project(2, "v", x2_s), 10, [norm] + prepare("w1", 1, range(5, 8)) + [sums]),
                 (q, 2, None),
                 (ffn1(a_s, 0), 12, arrival("w2") + v_transpose(2) + prepare("w2") + prepare("w2", 1, range(2))),
                 (ffn1(a_s, 1), 12, a_operands(a_s[0]) + prepare("w2", 1, range(2, 7))),
                 (q, 8, a_operands(a_s[1]) + prepare("w2", 1, range(7, 8)))], SCHEDULE_1)

    def body(t):
        step(t, [(ffn2(t - 2, a_s), 24, o_operands() + x_operands(t + 1, x_s)),
                 (out_proj(t - 1), 10, ()),
                 (project(t + 1, "k"), 10, h_operands()),
                 (project(t + 1, "v"), 10, None),
                 (ffn1(a_s, 0), 12, v_transpose(t + 1)),
                 (ffn1(a_s, 1), 12, a_operands(a_s[0])),
                 (project(t + 1, "q"), 10, a_operands(a_s[1]))], SCHEDULE_LOOP)

    def epilogue():
        t = NS - 1
        fa = ffn2(t - 2, a_s)
        fb = ffn2(t - 1, b_s, 1, stored=lambda c: o_copy(t - 2, 2, c).start())
        fc = ffn2(t, a_s, 0, ((0,), (1,)), lambda c: o_copy(t, 1, c).start())
        step(t, [(fa, 5, o_operands()), (out_proj(t - 1, 1), 10, ()), (fa, 11, h_operands(1)),
                 (ffn1(b_s, 0), 12, ()), (ffn1(b_s, 1), 12, a_operands(b_s[0])), (fa, 8, a_operands(b_s[1])),
                 (fb, 6, o_operands()), (out_proj(t), 10, ()), (fb, 18, h_operands()),
                 (ffn1(a_s, 0), 12, ()), (ffn1(a_s, 1), 12, a_operands(a_s[0])),
                 (fc, 12, a_operands(a_s[1])), (fc, 12, ())], SCHEDULE_END, after=24 + 10 + 24 + 24)

    def recompute():
        n = 32

        def tokens(i):
            words = [x_words(0, c, i * (n // 2), n // 2) for c in ALL]
            return _bf(jnp.concatenate(words, 1)).astype(F32)

        def matrix(name):
            return _bf(weights[name][0:(DFF if name == "w2" else D) // 2, :])

        @pl.loop(0, S // n)
        def _(i):
            xn = _normed(tokens(i)).astype(BF)
            for m, name in enumerate("qkv"):
                qkv_s[m, rows(i * n, n), :] = _dot(xn, matrix(name)).astype(BF)

        @pl.loop(0, S // n)
        def _(i):
            first = jnp.maximum((i * n) // 128 - 2, 0) * 128
            ahead = (i * n - first + lax.broadcasted_iota(I32, (n, 384), 0)
                     - lax.broadcasted_iota(I32, (n, 384), 1))
            lane = lax.broadcasted_iota(I32, (n, D), 1)

            def head(h, o):
                mine = (lane >= DH * h) & (lane < DH * h + DH)
                q = jnp.where(mine, qkv_s[0, rows(i * n, n), :].astype(F32), 0.0).astype(BF)
                s = _dot(q, qkv_s[1, rows(first, 384), :], NT) * (DH ** -0.5)
                s = jnp.where((ahead >= 0) & (ahead < 256), s, -1e9)
                p = jnp.exp(s - jnp.max(s, axis=-1, keepdims=True))
                p = p / jnp.sum(p, axis=-1, keepdims=True)
                return jnp.where(mine, _dot(p.astype(BF), qkv_s[2, rows(first, 384), :]), o)

            o = lax.fori_loop(0, H, head, jnp.zeros((n, D), F32))
            h = tokens(i) + _dot(o.astype(BF), matrix("o"))
            a = jnp.maximum(_dot(_normed(h).astype(BF), matrix("w1")), 0.0)
            out_s[rows(i * n, n, n), :] = (h + _dot(a.astype(BF), matrix("w2"))).astype(BF)

    def finale():
        start([o_copy(0, NS - 3, c) for c in ALL])
        epilogue()
        results = [o_copy(t, n, c) for t, n in ((0, NS - 3), (NS - 3, 2), (NS - 1, 1)) for c in ALL]
        inside = (range_s[0:1, :] >= 1.0 / RANGE) & (range_s[8:9, :] <= RANGE)

        @pl.when(jnp.sum(jnp.where(inside, 0.0, 1.0)) > 0.0)
        def _():
            wait(results)
            recompute()
            start(results)

        wait(results)

    pl.loop(zero, 1)(lambda _: prologue())
    wait(x_copies(3))
    pl.loop(2, NS - 1)(body)
    pl.loop(zero, 1)(lambda _: finale())


@jax.jit
def pallas_sequential_preLN__sliding_block__dense_activation_relu__prompt_kernel(
    A_x: jax.Array,
    A_wqkv: jax.Array,
    A_wo: jax.Array,
    B_x: jax.Array,
    B_w1: jax.Array,
    B_w2: jax.Array,
):
    del B_x

    def words(n, width=128):
        return pltpu.VMEM((n + 32, width), U32)

    def stage(tiles, more=0):
        return words(len(BAND.order) * PR + tiles * T + more)

    hbm = pl.BlockSpec(memory_space=pltpu.HBM)
    out = pl.pallas_call(
        _kernel,
        out_shape=jax.ShapeDtypeStruct((S, D), BF),
        in_specs=[hbm] * 5,
        out_specs=hbm,
        scratch_shapes=[
            *[words(64 * 9, D)] * 4, words(64 * 13, DFF), words(64 * 30, D),
            stage(5, 5 * S // 2), stage(5), stage(5), stage(18, 32),
            [stage(6)] * 2, [stage(6)] * 2,
            pltpu.VMEM((64, 8, 128), U32),
            pltpu.VMEM((32, 128), F32),
            words(8 * S // 2), words(8 * S),
            words(5 * HT),
            pltpu.VMEM((H * S // 4, 128), F32),
            pltpu.VMEM((2, D, 128), F32),
            pltpu.VMEM((S, D), BF),
            [words(4 * 208)] * 4,
            pltpu.VMEM((3, S, D), BF),
            pltpu.SemaphoreType.DMA((7,)), pltpu.SemaphoreType.DMA((4,)), pltpu.SemaphoreType.DMA(()),
            pltpu.SemaphoreType.REGULAR,
        ],
        compiler_params=pltpu.CompilerParams(vmem_limit_bytes=100 * 1024 * 1024),
        name="fused_block",
    )(A_x.reshape(S, D), A_wqkv, A_wo, B_w1, B_w2)
    return out.reshape(1, S, D)
```
